```python
import os as _os
_os.environ.setdefault("JAX_PLATFORMS", "cpu")
import jax
import jax.numpy as jnp

def _softmax(x, axis=-1):
    return jax.nn.softmax(x, axis=axis)
def _gelu(x):
    return jax.nn.gelu(x, approximate=True)
def _silu(x):
    return jax.nn.silu(x)
def _sigmoid(x):
    return jax.nn.sigmoid(x)
def _layernorm(x, axis=-1, eps=1e-5):
    m = jnp.mean(x, axis=axis, keepdims=True)
    v = jnp.var(x, axis=axis, keepdims=True)
    return (x - m) / jnp.sqrt(v + eps)
def _scatter_add(tgt, idx, src, axis=0):
    return tgt.at[idx].add(src)
def _segment_sum(src, seg, n):
    return jax.ops.segment_sum(src, seg, n)
class _Rng:
    def __init__(self, key):
        self._k = key
    def _next(self):
        self._k, sub = jax.random.split(self._k)
        return sub
    def normal(self, shape):
        return jax.random.normal(self._next(), shape, dtype=jnp.bfloat16)
    def randint(self, lo, hi, shape):
        return jax.random.randint(self._next(), shape, lo, hi, dtype=jnp.int32)
    def uniform(self, shape, lo=0.0, hi=1.0):
        return jax.random.uniform(self._next(), shape, jnp.bfloat16, lo, hi)
    def permutation(self, n):
        return jax.random.permutation(self._next(), n)


kernel_name = 'concat_heads__mha_block_cached__mha_block_cached__near_ridge'

def setup_inputs():
    _rng = _Rng(jax.random.key(int.from_bytes(__import__("os").urandom(4), "little")))
    _w = (lambda a: (lambda t: t.astype(jnp.bfloat16) if jnp.issubdtype(t.dtype, jnp.floating) else t)(jnp.asarray(a)))
    def _A_setup():
        B, Sq, D = 8, 160, 512
        H, Sk, Dh = 32, 512, 128
        return {
            "x": _w((lambda *s: _rng.normal(s) * 0.8)(B, Sq, D)),
            "k_cache": _w((lambda *s: _rng.normal(s) * 0.8)(B, H, Sk, Dh)),
            "v_cache": _w((lambda *s: _rng.normal(s) * 0.05)(B, H, Sk, Dh)),
            "wq": _w((lambda *s: _rng.normal(s) * 0.8)(D, H * Dh) * (D ** -0.5)),
            "wo": _w((lambda *s: _rng.normal(s) * 0.05)(H * Dh, D) * ((H * Dh) ** -0.5)),
        }
    _A_in = _A_setup()

    def _B_setup():
        B, Sq, D = 8, 160, 512
        H, Sk, Dh = 32, 512, 128
        return {
            "x": _w((lambda *s: _rng.normal(s) * 0.8)(B, Sq, D)),
            "k_cache": _w((lambda *s: _rng.normal(s) * 0.8)(B, H, Sk, Dh)),
            "v_cache": _w((lambda *s: _rng.normal(s) * 0.05)(B, H, Sk, Dh)),
            "wq": _w((lambda *s: _rng.normal(s) * 0.8)(D, H * Dh) * (D ** -0.5)),
            "wo": _w((lambda *s: _rng.normal(s) * 0.05)(H * Dh, D) * ((H * Dh) ** -0.5)),
        }
    _B_in = _B_setup()

    return {
        "A_x": _A_in["x"],
        "A_k_cache": _A_in["k_cache"],
        "A_v_cache": _A_in["v_cache"],
        "A_wq": _A_in["wq"],
        "A_wo": _A_in["wo"],
        "B_x": _B_in["x"],
        "B_k_cache": _B_in["k_cache"],
        "B_v_cache": _B_in["v_cache"],
        "B_wq": _B_in["wq"],
        "B_wo": _B_in["wo"],
    }

def reference(A_x, A_k_cache, A_v_cache, A_wq, A_wo, B_x, B_k_cache, B_v_cache, B_wq, B_wo):
    def _A_ref(x, k_cache, v_cache, wq, wo):
        B, Sq, D = x.shape
        H, Dh = 32, 128
        q = (lambda x, *d: x.transpose(*d))((x @ wq).reshape(B, Sq, H, Dh), 0, 2, 1, 3)
        scores = jnp.einsum("bhqd,bhkd->bhqk", q, k_cache) * (Dh ** -0.5)
        p = _softmax(scores, axis=-1)
        o = jnp.einsum("bhqk,bhkd->bhqd", p, v_cache)
        return (lambda x, *d: x.transpose(*d))(o, 0, 2, 1, 3).reshape(B, Sq, H * Dh) @ wo

    def _B_ref(x, k_cache, v_cache, wq, wo):
        B, Sq, D = x.shape
        H, Dh = 32, 128
        q = (lambda x, *d: x.transpose(*d))((x @ wq).reshape(B, Sq, H, Dh), 0, 2, 1, 3)
        scores = jnp.einsum("bhqd,bhkd->bhqk", q, k_cache) * (Dh ** -0.5)
        p = _softmax(scores, axis=-1)
        o = jnp.einsum("bhqk,bhkd->bhqd", p, v_cache)
        return (lambda x, *d: x.transpose(*d))(o, 0, 2, 1, 3).reshape(B, Sq, H * Dh) @ wo

    a = _A_ref(A_x, A_k_cache, A_v_cache, A_wq, A_wo)
    b = _B_ref(B_x, B_k_cache, B_v_cache, B_wq, B_wo)
    return jnp.concatenate([a, b], axis=-1)
```

```python
import functools

import jax
import jax.numpy as jnp
from jax import lax
import jax.experimental.pallas as pl
import jax.experimental.pallas.tpu as pltpu

HG = 8


def _branch(x_ref, k_ref, v_ref, wq_ref, wo_ref, hg, dh):
    scale = dh ** -0.5
    x = x_ref[0]
    q = (jnp.dot(x, wq_ref[...], preferred_element_type=jnp.float32) * scale).astype(jnp.bfloat16)
    outs = []
    for h in range(hg):
        qh = q[:, h * dh:(h + 1) * dh]
        s = lax.dot_general(qh, k_ref[0, h], (((1,), (1,)), ((), ())),
                            preferred_element_type=jnp.float32)
        m = jnp.max(s, axis=-1, keepdims=True)
        p = jnp.exp(s - m)
        l = jnp.sum(p, axis=-1, keepdims=True)
        oh = jnp.dot(p.astype(jnp.bfloat16), v_ref[0, h], preferred_element_type=jnp.float32)
        outs.append((oh / l).astype(jnp.bfloat16))
    o = jnp.concatenate(outs, axis=1)
    return jnp.dot(o, wo_ref[...], preferred_element_type=jnp.float32)


def _kernel(xa, ka, va, wqa, woa, xb, kb, vb, wqb, wob, o_ref, acc_ref, *, hg, dh, d):
    g = pl.program_id(0)
    b = pl.program_id(1)
    ng = pl.num_programs(0)
    ca = _branch(xa, ka, va, wqa, woa, hg, dh)
    cb = _branch(xb, kb, vb, wqb, wob, hg, dh)

    @pl.when(g == 0)
    def _():
        acc_ref[b, :, 0:d] = ca
        acc_ref[b, :, d:2 * d] = cb

    @pl.when(jnp.logical_and(g > 0, g < ng - 1))
    def _():
        acc_ref[b, :, 0:d] += ca
        acc_ref[b, :, d:2 * d] += cb

    @pl.when(g == ng - 1)
    def _():
        o_ref[b, :, 0:d] = (acc_ref[b, :, 0:d] + ca).astype(o_ref.dtype)
        o_ref[b, :, d:2 * d] = (acc_ref[b, :, d:2 * d] + cb).astype(o_ref.dtype)


@jax.jit
def pallas_concat_heads__mha_block_cached__mha_block_cached__near_ridge_kernel(
    A_x, A_k_cache, A_v_cache, A_wq, A_wo, B_x, B_k_cache, B_v_cache, B_wq, B_wo,
):
    B, Sq, D = A_x.shape
    _, H, Sk, Dh = A_k_cache.shape
    hg = HG
    ng = H // hg

    x_spec = pl.BlockSpec((1, Sq, D), lambda g, b: (b, 0, 0))
    kv_spec = pl.BlockSpec((1, hg, Sk, Dh), lambda g, b: (b, g, 0, 0))
    wq_spec = pl.BlockSpec((D, hg * Dh), lambda g, b: (0, g))
    wo_spec = pl.BlockSpec((hg * Dh, D), lambda g, b: (g, 0))
    specs = [x_spec, kv_spec, kv_spec, wq_spec, wo_spec]

    return pl.pallas_call(
        functools.partial(_kernel, hg=hg, dh=Dh, d=D),
        grid=(ng, B),
        in_specs=specs + specs,
        out_specs=pl.BlockSpec((B, Sq, 2 * D), lambda g, b: (0, 0, 0)),
        out_shape=jax.ShapeDtypeStruct((B, Sq, 2 * D), A_x.dtype),
        scratch_shapes=[pltpu.VMEM((B, Sq, 2 * D), jnp.float32)],
        compiler_params=pltpu.CompilerParams(
            dimension_semantics=("arbitrary", "arbitrary"),
            vmem_limit_bytes=100 * 1024 * 1024,
        ),
    )(A_x, A_k_cache, A_v_cache, A_wq, A_wo, B_x, B_k_cache, B_v_cache, B_wq, B_wo)
```

```python
import functools

import jax
import jax.numpy as jnp
from jax import lax
import jax.experimental.pallas as pl
import jax.experimental.pallas.tpu as pltpu

HG = 8
LA = 1


def _kernel(xa, ka, va, wqa, woa, xb, kb, vb, wqb, wob, o_hbm,
            kvbuf, wqbuf, wobuf, acc_ref, obuf, kv_sem, w_sem, o_sem, *, hg, dh, d, nb, ng):
    g = pl.program_id(0)
    b = pl.program_id(1)
    t = g * nb + b
    nt = ng * nb
    slot = t % 3
    wslot = g % 2
    scale = dh ** -0.5
    kv_hbm = ((ka, va), (kb, vb))
    w_hbm = ((wqa, woa), (wqb, wob))
    xs = (xa, xb)

    def kv_copy(gg, bb, sl, br, which):
        return pltpu.make_async_copy(kv_hbm[br][which].at[bb, pl.ds(gg * hg, hg)],
                                     kvbuf.at[sl, br, which], kv_sem.at[sl, br, which])

    def w_copy(gg, sl, br, which):
        if which == 0:
            return pltpu.make_async_copy(w_hbm[br][0].at[:, pl.ds(gg * (hg * dh), hg * dh)],
                                         wqbuf.at[sl, br], w_sem.at[sl, br, 0])
        return pltpu.make_async_copy(w_hbm[br][1].at[pl.ds(gg * (hg * dh), hg * dh), :],
                                     wobuf.at[sl, br], w_sem.at[sl, br, 1])

    def o_copy(bb):
        return pltpu.make_async_copy(obuf.at[bb], o_hbm.at[bb], o_sem.at[bb])

    @pl.when(t == 0)
    def _():
        w_copy(0, 0, 0, 0).start()
        w_copy(0, 0, 1, 0).start()
        w_copy(0, 0, 0, 1).start()
        w_copy(0, 0, 1, 1).start()
        for br in range(2):
            for which in range(2):
                kv_copy(0, 0, 0, br, which).start()
        acc_ref[...] = jnp.zeros(acc_ref.shape, acc_ref.dtype)

    @pl.when(jnp.logical_and(b == 1, g + 1 < ng))
    def _():
        for br in range(2):
            for which in range(2):
                w_copy(g + 1, 1 - wslot, br, which).start()

    @pl.when(b == 0)
    def _():
        for br in range(2):
            for which in range(2):
                w_copy(g, wslot, br, which).wait()

    for br in range(2):
        for which in range(2):
            kv_copy(g, b, slot, br, which).wait()

    @pl.when(t == 0)
    def _():
        for br in range(2):
            for which in range(2):
                kv_copy(0, 1, 1, br, which).start()

    @pl.when(t + 2 < nt)
    def _():
        nb_ = (b + 2) % nb
        ng_ = g + (b + 2) // nb
        for br in range(2):
            for which in range(2):
                kv_copy(ng_, nb_, (t + 2) % 3, br, which).start()

    def qproj(br):
        return (jnp.dot(xs[br][0], wqbuf[wslot, br], preferred_element_type=jnp.float32) * scale).astype(jnp.bfloat16)

    qs = [qproj(0), None]
    waited = set()

    def kv(br, which, h):
        return kvbuf[slot, br, which, h]

    def qk(i):
        br, h = divmod(i, hg)
        if qs[br] is None:
            qs[br] = qproj(br)
        return lax.dot_general(qs[br][:, h * dh:(h + 1) * dh], kv(br, 0, h), (((1,), (1,)), ((), ())),
                               preferred_element_type=jnp.float32)

    n = 2 * hg
    pend = [qk(i) for i in range(LA)]
    outs = []
    for i in range(n):
        br, h = divmod(i, hg)
        if i + LA < n:
            pend.append(qk(i + LA))
        s = pend.pop(0)
        m = jnp.max(s, axis=-1, keepdims=True)
        p = jnp.exp(s - m)
        l = jnp.sum(p, axis=-1, keepdims=True)
        oh = jnp.dot(p.astype(jnp.bfloat16), kv(br, 1, h), preferred_element_type=jnp.float32)
        r = pl.reciprocal(l, approx=True)
        r = r * (2.0 - l * r)
        outs.append((oh * r).astype(jnp.bfloat16))
        if h == hg - 1:
            o = jnp.concatenate(outs, axis=1)
            outs = []
            acc_ref[b, :, br * d:(br + 1) * d] += jnp.dot(o, wobuf[wslot, br], preferred_element_type=jnp.float32)

    @pl.when(g == ng - 1)
    def _():
        obuf[b] = acc_ref[b].astype(obuf.dtype)
        o_copy(b).start()

    @pl.when(t == nt - 1)
    def _():
        for bb in range(nb):
            o_copy(bb).wait()


@jax.jit
def pallas_concat_heads__mha_block_cached__mha_block_cached__near_ridge_kernel(
    A_x, A_k_cache, A_v_cache, A_wq, A_wo, B_x, B_k_cache, B_v_cache, B_wq, B_wo,
):
    B, Sq, D = A_x.shape
    _, H, Sk, Dh = A_k_cache.shape
    hg = HG
    ng = H // hg
    dt = A_x.dtype

    x_spec = pl.BlockSpec((1, Sq, D), lambda g, b: (b, 0, 0))
    any_spec = pl.BlockSpec(memory_space=pl.ANY)
    specs = [x_spec, any_spec, any_spec, any_spec, any_spec]

    return pl.pallas_call(
        functools.partial(_kernel, hg=hg, dh=Dh, d=D, nb=B, ng=ng),
        grid=(ng, B),
        in_specs=specs + specs,
        out_specs=any_spec,
        out_shape=jax.ShapeDtypeStruct((B, Sq, 2 * D), dt),
        scratch_shapes=[
            pltpu.VMEM((3, 2, 2, hg, Sk, Dh), dt),
            pltpu.VMEM((2, 2, D, hg * Dh), dt),
            pltpu.VMEM((2, 2, hg * Dh, D), dt),
            pltpu.VMEM((B, Sq, 2 * D), jnp.float32),
            pltpu.VMEM((B, Sq, 2 * D), dt),
            pltpu.SemaphoreType.DMA((3, 2, 2)),
            pltpu.SemaphoreType.DMA((2, 2, 2)),
            pltpu.SemaphoreType.DMA((B,)),
        ],
        compiler_params=pltpu.CompilerParams(
            dimension_semantics=("arbitrary", "arbitrary"),
            vmem_limit_bytes=100 * 1024 * 1024,
        ),
    )(A_x, A_k_cache, A_v_cache, A_wq, A_wo, B_x, B_k_cache, B_v_cache, B_wq, B_wo)
```
